```python
import jax
import jax.numpy as jnp

def _softmax(x, axis=-1):
    return jax.nn.softmax(x, axis=axis)
def _gelu(x):
    return jax.nn.gelu(x, approximate=True)
def _silu(x):
    return jax.nn.silu(x)
def _sigmoid(x):
    return jax.nn.sigmoid(x)
def _layernorm(x, axis=-1, eps=1e-5):
    m = jnp.mean(x, axis=axis, keepdims=True)
    v = jnp.var(x, axis=axis, keepdims=True)
    return (x - m) / jnp.sqrt(v + eps)
def _scatter_add(tgt, idx, src, axis=0):
    return tgt.at[idx].add(src)
def _segment_sum(src, seg, n):
    return jax.ops.segment_sum(src, seg, n)
class _Rng:
    def __init__(self, key):
        self._k = key
    def _next(self):
        self._k, sub = jax.random.split(self._k)
        return sub
    def normal(self, shape):
        return jax.random.normal(self._next(), shape, dtype=jnp.bfloat16)
    def randint(self, lo, hi, shape):
        return jax.random.randint(self._next(), shape, lo, hi, dtype=jnp.int32)
    def uniform(self, shape, lo=0.0, hi=1.0):
        return jax.random.uniform(self._next(), shape, jnp.bfloat16, lo, hi)
    def permutation(self, n):
        return jax.random.permutation(self._next(), n)


kernel_name = 'concat_heads__compressed_kv_cla__mha_block_cached__decode'

def setup_inputs():
    _rng = _Rng(jax.random.key(int.from_bytes(__import__("os").urandom(4), "little")))
    _w = (lambda a: (lambda t: t.astype(jnp.bfloat16) if jnp.issubdtype(t.dtype, jnp.floating) else t)(jnp.asarray(a)))
    def _A_setup():
        B, H, Sq, Sk, D, M = 4, 32, 1, 4096, 128, 512
        Dc = 4 * D
        return {
            "x": _w((lambda *s: _rng.normal(s) * 0.05)(B, Sq, M)),
            "c_kv": _w((lambda *s: _rng.normal(s) * 0.05)(B, Sk, Dc)),
            "w_q": _w((lambda *s: _rng.normal(s) * 0.05)(M, H, D) * (M ** -0.5)),
            "w_uk": _w((lambda *s: _rng.normal(s) * 0.05)(Dc, H, D) * (Dc ** -0.5)),
            "w_uv": _w((lambda *s: _rng.normal(s) * 0.05)(Dc, H, D) * (Dc ** -0.5)),
            "w_o": _w((lambda *s: _rng.normal(s) * 0.05)(H, D, M) * ((H * D) ** -0.5)),
        }
    _A_in = _A_setup()

    def _B_setup():
        B, Sq, D = 4, 1, 512
        H, Sk, Dh = 32, 4096, 128
        return {
            "x": _w((lambda *s: _rng.normal(s) * 0.05)(B, Sq, D)),
            "k_cache": _w((lambda *s: _rng.normal(s) * 0.05)(B, H, Sk, Dh)),
            "v_cache": _w((lambda *s: _rng.normal(s) * 0.05)(B, H, Sk, Dh)),
            "wq": _w((lambda *s: _rng.normal(s) * 0.05)(D, H * Dh) * (D ** -0.5)),
            "wo": _w((lambda *s: _rng.normal(s) * 0.05)(H * Dh, D) * ((H * Dh) ** -0.5)),
        }
    _B_in = _B_setup()

    return {
        "A_x": _A_in["x"],
        "A_c_kv": _A_in["c_kv"],
        "A_w_q": _A_in["w_q"],
        "A_w_uk": _A_in["w_uk"],
        "A_w_uv": _A_in["w_uv"],
        "A_w_o": _A_in["w_o"],
        "B_x": _B_in["x"],
        "B_k_cache": _B_in["k_cache"],
        "B_v_cache": _B_in["v_cache"],
        "B_wq": _B_in["wq"],
        "B_wo": _B_in["wo"],
    }

def reference(A_x, A_c_kv, A_w_q, A_w_uk, A_w_uv, A_w_o, B_x, B_k_cache, B_v_cache, B_wq, B_wo):
    def _A_ref(x, c_kv, w_q, w_uk, w_uv, w_o):
        B, Sq, M = x.shape[0], x.shape[1], x.shape[2]
        Sk = c_kv.shape[1]
        H, D = w_q.shape[1], w_q.shape[2]
        q = jnp.einsum("bqm,mhd->bhqd", x, w_q)
        k = jnp.einsum("bkc,chd->bhkd", c_kv, w_uk)
        v = jnp.einsum("bkc,chd->bhkd", c_kv, w_uv)
        scores = jnp.einsum("bhqd,bhkd->bhqk", q, k) * (D ** -0.5)
        off = Sk - Sq
        qi = jnp.arange(Sq)[:, None]
        kj = jnp.arange(Sk)[None, :]
        cmask = kj <= (qi + off)
        scores = jnp.where(cmask[None, None], scores, -1e9)
        p = _softmax(scores, axis=-1)
        ctx = jnp.einsum("bhqk,bhkd->bhqd", p, v)
        return jnp.einsum("bhqd,hdm->bqm", ctx, w_o)

    def _B_ref(x, k_cache, v_cache, wq, wo):
        B, Sq, D = x.shape
        H, Dh = 32, 128
        q = (lambda x, *d: x.transpose(*d))((x @ wq).reshape(B, Sq, H, Dh), 0, 2, 1, 3)
        scores = jnp.einsum("bhqd,bhkd->bhqk", q, k_cache) * (Dh ** -0.5)
        p = _softmax(scores, axis=-1)
        o = jnp.einsum("bhqk,bhkd->bhqd", p, v_cache)
        return (lambda x, *d: x.transpose(*d))(o, 0, 2, 1, 3).reshape(B, Sq, H * Dh) @ wo

    a = _A_ref(A_x, A_c_kv, A_w_q, A_w_uk, A_w_uv, A_w_o)
    b = _B_ref(B_x, B_k_cache, B_v_cache, B_wq, B_wo)
    return jnp.concatenate([a, b], axis=-1)
```

```python
import functools

import jax
import jax.numpy as jnp
from jax import lax
import jax.experimental.pallas as pl
import jax.experimental.pallas.tpu as pltpu

_NT = (((1,), (1,)), ((), ()))
_PIECES = 64
_UNROLL = 16
_AHEAD = 4
_SLOTS = _AHEAD // 2 + 1
_HG = 16
_F32 = jnp.float32
_BF16 = jnp.bfloat16


def _dot(a, b):
    return jnp.dot(a, b, preferred_element_type=_F32)


def _dot_nt(a, b):
    return lax.dot_general(a, b, _NT, preferred_element_type=_F32)


def _iota(shape, dim):
    return lax.broadcasted_iota(jnp.int32, shape, dim)


def _ds(start, size):
    return pl.ds(pl.multiple_of(start, size), size)


def _kernel(
    xa_hbm, ckv_hbm, wqa_hbm, wuk_hbm, wuv_hbm, woa_hbm,
    xb_hbm, k_hbm, v_hbm, wqb_hbm, wob_hbm,
    out_ref,
    xa_v, xb_v, wqa_v, wuk_v, ckv_v, wuv_v, woa_v, wqb_v, wob_v, k_v, v_v,
    e_s, et_s, xr_s, qabs_s, ctxc_s, ctx_s, qb_s, sems, xsems,
):
    nb, nh, sk, dh = k_hbm.shape
    dm = xa_hbm.shape[-1]
    ng = nh // _HG
    rows = nb * _HG
    wide = 128 * _HG
    kblk = sk // 4
    scale = dh ** -0.5

    def up_phase(hbm, vmem):
        n = 128 // _PIECES

        def piece(j, u):
            sl = _ds(j * 128 + u * n, n)
            return hbm.at[sl], vmem.at[sl]

        return piece, lambda j: vmem.at[_ds(j * 128, 128)]

    def ckv_piece(j, u):
        n = kblk // _PIECES
        sl = _ds((j % 4) * kblk + u * n, n)
        return ckv_hbm.at[j // 4, sl], ckv_v.at[j // 4, sl]

    def woa_piece(j, u):
        per = _PIECES // 8
        n = dh // per
        sl = _ds((u % per) * n, n)
        return woa_hbm.at[j * 8 + u // per, sl], woa_v.at[j * 8 + u // per, sl]

    def wqb_piece(j, u):
        n = 2 * dm // _PIECES
        r = _ds((u // 2) * n, n)
        return (wqb_hbm.at[r, _ds(j * 1024 + (u % 2) * 512, 512)],
                wqb_v.at[j, r, _ds((u % 2) * 512, 512)])

    def wob_piece(j, u):
        n = 1024 // _PIECES
        sl = _ds(j * 1024 + u * n, n)
        return wob_hbm.at[sl], wob_v.at[sl]

    def cache_phase(hbm, vmem):
        n = sk // _PIECES

        def piece(i, u):
            sl = _ds(u * n, n)
            return hbm.at[i // nh, i % nh, sl], vmem.at[i % _SLOTS, sl]

        return piece, lambda i: vmem.at[i % _SLOTS]

    p_wqa = up_phase(wqa_hbm, wqa_v)
    p_wuk = up_phase(wuk_hbm, wuk_v)
    p_ckv = (ckv_piece, lambda j: ckv_v.at[j // 4, _ds((j % 4) * kblk, kblk)])
    p_wuv = up_phase(wuv_hbm, wuv_v)
    p_woa = (woa_piece, lambda j: woa_v.at[_ds(j * 8, 8)])
    p_wqb = (wqb_piece, lambda j: wqb_v.at[j])
    p_wob = (wob_piece, lambda j: wob_v.at[_ds(j * 1024, 1024)])
    p_cache = (cache_phase(k_hbm, k_v), cache_phase(v_hbm, v_v))

    order = ((p_wqa, 4), (p_wuk, 4), (p_ckv, 4 * nb), (p_wuv, 4), (p_woa, 4),
             (p_wqb, 4), (p_wob, 4))
    first = [sum(n for _, n in order[:k]) for k in range(len(order) + 1)]
    n_wqa, n_wuk, n_ckv, n_wuv, n_woa, n_wqb, n_wob, n_cache = first

    def issue(phase, j, n):
        def body(t, carry):
            for r in range(_UNROLL):
                src, dst = phase[0](j, t * _UNROLL + r)
                pltpu.make_async_copy(src, dst, sems.at[n % _AHEAD]).start(priority=r % 2)
            return carry

        lax.fori_loop(0, _PIECES // _UNROLL, body, None)

    def wait(phase, j, n):
        dst = phase[1](j)
        pltpu.make_async_copy(dst, dst, sems.at[n % _AHEAD]).wait()

    def issue_block(n, lo, hi):
        for (phase, size), start in zip(order, first):
            if lo >= start and hi <= start + size:
                issue(phase, n - start, n)
            elif lo < start + size and hi > start:
                pl.when((n >= start) & (n < start + size))(
                    functools.partial(issue, phase, n - start, n))
        if hi > n_cache:
            t = n - n_cache
            for kv in range(2):
                pl.when((t >= 0) & (t % 2 == kv))(
                    functools.partial(issue, p_cache[kv], t // 2, n))

    def issue_ahead(start, size, j):
        issue_block(start + j + _AHEAD, start + _AHEAD, start + size + _AHEAD)

    xa_cp = pltpu.make_async_copy(xa_hbm, xa_v, xsems.at[0])
    xb_cp = pltpu.make_async_copy(xb_hbm, xb_v, xsems.at[1])
    xa_cp.start()
    xb_cp.start()
    issue(p_wqa, 0, 0)

    e_s[...] = (_iota((128, wide), 1) // _HG == _iota((128, wide), 0)).astype(_BF16)
    et_s[...] = (_iota((wide, 128), 0) // _HG == _iota((wide, 128), 1)).astype(_BF16)
    xa_cp.wait()
    xb_cp.wait()
    xa = xa_v[...].astype(_F32)
    for b in range(nb):
        xrow = jnp.broadcast_to(xa[b:b + 1], (_HG, dm)).astype(_BF16)
        for i in range(dm // 128):
            xr_s[i, b * _HG:(b + 1) * _HG, :] = xrow[:, i * 128:(i + 1) * 128]

    for n in range(1, _AHEAD):
        issue_block(n, n, n + 1)

    def own_head(t):
        keep = _iota((rows, wide), 0) % _HG == _iota((rows, wide), 1) % _HG
        return jnp.where(keep, t, 0.0).astype(_BF16)

    def group_rows(w_v, j, g):
        return w_v[_ds(j * 128, 128), g * _HG:(g + 1) * _HG, :].reshape(wide, dh)

    zeros_q = tuple(jnp.zeros((rows, dh), _F32) for _ in range(ng))

    def qa_step(j, q):
        wait(p_wqa, j, n_wqa + j)
        lhs = own_head(_dot(xr_s[j], e_s[...]))
        q = tuple(q[g] + _dot(lhs, group_rows(wqa_v, j, g)) for g in range(ng))
        issue_ahead(n_wqa, 4, j)
        return q

    qa = lax.fori_loop(0, 4, qa_step, zeros_q)
    qa = tuple(q.astype(_BF16) for q in qa)

    def qabs_step(j, carry):
        wait(p_wuk, j, n_wuk + j)
        for g in range(ng):
            t = own_head(_dot_nt(qa[g], group_rows(wuk_v, j, g)))
            t = _dot(t, et_s[...]).astype(_BF16)
            for b in range(nb):
                qabs_s[j, b, g * _HG:(g + 1) * _HG, :] = t[b * _HG:(b + 1) * _HG]
        issue_ahead(n_wuk, 4, j)
        return carry

    lax.fori_loop(0, 4, qabs_step, None)

    def latent_batch(b, carry):
        q = jnp.concatenate([qabs_s[i, b] for i in range(4)], axis=-1)

        def step(jj, state):
            m, l, acc = state
            j = b * 4 + jj
            wait(p_ckv, j, n_ckv + j)
            c = ckv_v[b, _ds(jj * kblk, kblk), :]
            s = _dot_nt(q, c) * scale
            m_new = jnp.maximum(m, jnp.max(s, axis=-1, keepdims=True))
            alpha = jnp.exp(m - m_new)
            p = jnp.exp(s - m_new)
            l = alpha * l + jnp.sum(p, axis=-1, keepdims=True)
            acc = alpha * acc + _dot(p.astype(_BF16), c)
            issue_ahead(n_ckv, 4 * nb, j)
            return m_new, l, acc

        init = (jnp.full((nh, 1), -jnp.inf, _F32), jnp.zeros((nh, 1), _F32),
                jnp.zeros((nh, ckv_v.shape[-1]), _F32))
        _, l, acc = lax.fori_loop(0, 4, step, init)
        ctxc = (acc / l).astype(_BF16)
        for i in range(4):
            for g in range(ng):
                ctxc_s[i, g, _ds(b * _HG, _HG), :] = (
                    ctxc[g * _HG:(g + 1) * _HG, i * 128:(i + 1) * 128])
        return carry

    lax.fori_loop(0, nb, latent_batch, None)

    def ctx_step(j, ctx):
        wait(p_wuv, j, n_wuv + j)
        ctx = tuple(
            ctx[g] + _dot(own_head(_dot(ctxc_s[j, g], e_s[...])), group_rows(wuv_v, j, g))
            for g in range(ng))
        issue_ahead(n_wuv, 4, j)
        return ctx

    ctx = lax.fori_loop(0, 4, ctx_step, zeros_q)
    for g in range(ng):
        ctx_s[g] = ctx[g]

    def outa_step(j, acc):
        wait(p_woa, j, n_woa + j)
        shape = (rows, 8 * dh)
        keep = _iota(shape, 0) % _HG == (j % 2) * 8 + _iota(shape, 1) // dh
        lhs = jnp.where(keep, jnp.concatenate([ctx_s[j // 2]] * 8, axis=-1), 0.0)
        acc = acc + _dot(lhs.astype(_BF16), woa_v[_ds(j * 8, 8)].reshape(8 * dh, dm))
        issue_ahead(n_woa, 4, j)
        return acc

    outa = lax.fori_loop(0, 4, outa_step, jnp.zeros((rows, dm), _F32))
    outa = jnp.sum(outa.reshape(nb, _HG, dm), axis=1)
    out_ref[:, 0:dm] = outa.astype(out_ref.dtype)

    xb_rows = xb_v[...].astype(_F32)
    xb = jnp.zeros((8, dm), _F32)
    for b in range(nb):
        xb = jnp.where(_iota((8, dm), 0) == b, xb_rows[b:b + 1], xb)
    xb = xb.astype(_BF16)

    def qb_step(j, carry):
        wait(p_wqb, j, n_wqb + j)
        q = _dot(xb, wqb_v[j])
        for h in range(8):
            qb_s[j * 8 + h] = q[:, h * dh:(h + 1) * dh]
        issue_ahead(n_wqb, 4, j)
        return carry

    lax.fori_loop(0, 4, qb_step, None)

    def wob_step(j, carry):
        wait(p_wob, j, n_wob + j)
        issue_ahead(n_wob, 4, j)
        return carry

    lax.fori_loop(0, 4, wob_step, None)

    def refill(t):
        def go(i):
            i_next = i + (t + _AHEAD) // 2
            pl.when(i_next < nb * nh)(lambda: issue(
                p_cache[(t + _AHEAD) % 2], i_next, n_cache + 2 * i + t))
        return go

    def head_step(i, acc):
        b, h = i // nh, i % nh
        wait(p_cache[0], i, n_cache + 2 * i)
        s = _dot_nt(qb_s[h].astype(_BF16), k_v[i % _SLOTS]) * scale
        p = jnp.exp(s - jnp.max(s, axis=-1, keepdims=True))
        l = jnp.sum(p, axis=-1, keepdims=True)
        p = p.astype(_BF16)
        refill(0)(i)
        wait(p_cache[1], i, n_cache + 2 * i + 1)
        o = _dot(p, v_v[i % _SLOTS]) / l
        o = jnp.where(_iota(o.shape, 0) == b, o, 0.0).astype(_BF16)
        acc = acc + _dot(o, wob_v[_ds(h * dh, dh), :])
        refill(1)(i)
        return acc

    outb = lax.fori_loop(0, nb * nh, head_step, jnp.zeros((8, dm), _F32))
    out_ref[:, dm:2 * dm] = outb[0:nb].astype(out_ref.dtype)


@jax.jit
def pallas_concat_heads__compressed_kv_cla__mha_block_cached__decode_kernel(
    A_x: jax.Array,
    A_c_kv: jax.Array,
    A_w_q: jax.Array,
    A_w_uk: jax.Array,
    A_w_uv: jax.Array,
    A_w_o: jax.Array,
    B_x: jax.Array,
    B_k_cache: jax.Array,
    B_v_cache: jax.Array,
    B_wq: jax.Array,
    B_wo: jax.Array,
):
    nb, sq, dm = A_x.shape
    _, nh, sk, dh = B_k_cache.shape
    assert (nb, sq, dm, nh, sk, dh) == (4, 1, 512, 32, 4096, 128)
    assert A_c_kv.shape == (nb, sk, 512) and A_w_q.shape == (dm, nh, dh)
    rows, wide = nb * _HG, 128 * _HG
    vmem = pltpu.VMEM
    out = pl.pallas_call(
        _kernel,
        out_shape=jax.ShapeDtypeStruct((nb, 2 * dm), A_x.dtype),
        in_specs=[pl.BlockSpec(memory_space=pltpu.HBM)] * 11,
        out_specs=pl.BlockSpec(memory_space=pltpu.VMEM),
        scratch_shapes=[
            vmem((nb, dm), _BF16),
            vmem((nb, dm), _BF16),
            vmem(A_w_q.shape, _BF16),
            vmem(A_w_uk.shape, _BF16),
            vmem(A_c_kv.shape, _BF16),
            vmem(A_w_uv.shape, _BF16),
            vmem(A_w_o.shape, _BF16),
            vmem((4, dm, 1024), _BF16),
            vmem(B_wo.shape, _BF16),
            vmem((_SLOTS, sk, dh), _BF16),
            vmem((_SLOTS, sk, dh), _BF16),
            vmem((128, wide), _BF16),
            vmem((wide, 128), _BF16),
            vmem((dm // 128, rows, 128), _BF16),
            vmem((4, nb, nh, 128), _BF16),
            vmem((4, nh // _HG, rows, 128), _BF16),
            vmem((nh // _HG, rows, dh), _F32),
            vmem((nh, 8, dh), _F32),
            pltpu.SemaphoreType.DMA((_AHEAD,)),
            pltpu.SemaphoreType.DMA((2,)),
        ],
        compiler_params=pltpu.CompilerParams(
            vmem_limit_bytes=100 * 2**20,
            disable_bounds_checks=True,
        ),
    )(A_x.reshape(nb, dm), A_c_kv, A_w_q, A_w_uk, A_w_uv, A_w_o,
      B_x.reshape(nb, dm), B_k_cache, B_v_cache, B_wq, B_wo)
    return out.reshape(nb, sq, 2 * dm)
```

```python
import functools

import jax
import jax.numpy as jnp
from jax import lax
import jax.experimental.pallas as pl
import jax.experimental.pallas.tpu as pltpu

_NT = (((1,), (1,)), ((), ()))
_PIECES = 64
_UNROLL = 32
_AHEAD = 4
_SLOTS = 8
_HG = 16
_KEYS = 128
_F32 = jnp.float32
_BF16 = jnp.bfloat16


def _dot(a, b):
    return jnp.dot(a, b, preferred_element_type=_F32)


def _dot_nt(a, b):
    return lax.dot_general(a, b, _NT, preferred_element_type=_F32)


def _iota(shape, dim):
    return lax.broadcasted_iota(jnp.int32, shape, dim)


def _ds(start, size):
    return pl.ds(pl.multiple_of(start, size), size)


def _own_chunk(t):
    head = _iota((t.shape[0], 128), 0) % 8
    out = t[:, 0:128]
    for h in range(1, 8):
        out = jnp.where(head == h, t[:, h * 128:(h + 1) * 128], out)
    return out


def _kernel(
    xa_hbm, ckv_hbm, wqa_hbm, wuk_hbm, wuv_hbm, woa_hbm,
    xb_hbm, k_hbm, v_hbm, wqb_hbm, wob_hbm,
    out_ref,
    xa_v, xb_v, wqa_v, wuk_v, ckv_v, wuv_v, woa_v, wqb_v, wob_v, kv_v,
    e_s, et_s, xr_s, qabs_s, ctxc_s, ctx_s, qb_s, sc_s, sems, xsems,
):
    nb, nh, sk, dh = k_hbm.shape
    dm = xa_hbm.shape[-1]
    ng = nh // _HG
    rows = nb * _HG
    wide = 128 * _HG
    nkb = sk // _KEYS
    scale = dh ** -0.5

    def up_piece(hbm, vmem):
        def piece(j, t, r):
            u = t * (_UNROLL // 2) + r // 2
            sl = _ds(j * 128 + (r % 2) * 64 + u * 2, 2)
            return hbm.at[sl], vmem.at[sl]

        return piece

    def ckv_piece(j, t, r):
        u = t * (_UNROLL // 8) + r // 8
        src = _ds((r % 8) * 512 + (j % 4) * 128 + u * 16, 16)
        return ckv_hbm.at[j // 4, src], ckv_v.at[j, _ds((r % 8) * 128 + u * 16, 16)]

    def out_piece(hbm, vmem):
        def piece(j, t, r):
            sl = _ds((t * (_UNROLL // 8) + r // 8) * 16, 16)
            return hbm.at[(r % 8) * 4 + j, sl], vmem.at[j, r % 8, sl]

        return piece

    def wqb_piece(j, t, r):
        u = t * (_UNROLL // 8) + r // 8
        sl = _ds((r % 8) * 64 + (u // 2) * 16, 16)
        return (wqb_hbm.at[sl, _ds(j * 1024 + (u % 2) * 512, 512)],
                wqb_v.at[j, sl, _ds((u % 2) * 512, 512)])

    def cache_piece(hbm):
        def piece(j, t, r):
            n = _KEYS * nh // _PIECES
            u = t * (_UNROLL // nh) + r // nh
            src = _ds((j % nkb) * _KEYS + u * n, n)
            return (hbm.at[j // (2 * nkb), r % nh, src],
                    kv_v.at[j % _SLOTS, r % nh, _ds(u * n, n)])

        return piece

    def start(piece, j, n):
        def body(t, carry):
            for r in range(_UNROLL):
                src, dst = piece(j, t, r)
                pltpu.make_async_copy(src, dst, sems.at[n % _AHEAD]).start(priority=r % 2)
            return carry

        lax.fori_loop(0, _PIECES // _UNROLL, body, None)

    def start_cache(j, n):
        is_k = (j // nkb) % 2 == 0
        pl.when(is_k)(lambda: start(cache_piece(k_hbm), j, n))
        pl.when(jnp.logical_not(is_k))(lambda: start(cache_piece(v_hbm), j, n))

    phases = (
        (4, functools.partial(start, up_piece(wqa_hbm, wqa_v))),
        (4, functools.partial(start, up_piece(wuk_hbm, wuk_v))),
        (4 * nb, functools.partial(start, ckv_piece)),
        (4, functools.partial(start, up_piece(wuv_hbm, wuv_v))),
        (4, functools.partial(start, out_piece(woa_hbm, woa_v))),
        (4, functools.partial(start, wqb_piece)),
        (2 * nkb * nb, start_cache),
        (4, functools.partial(start, out_piece(wob_hbm, wob_v))),
    )
    first = [sum(size for size, _ in phases[:k]) for k in range(len(phases))]
    n_wqa, n_wuk, n_ckv, n_wuv, n_woa, n_wqb, n_cache, n_wob = first

    def start_block(n, lo, hi):
        for (size, start_phase), n0 in zip(phases, first):
            if lo >= n0 and hi <= n0 + size:
                start_phase(n - n0, n)
            elif lo < n0 + size and hi > n0:
                pl.when((n >= n0) & (n < n0 + size))(
                    functools.partial(start_phase, n - n0, n))

    def refill(n0, size, j):
        start_block(n0 + j + _AHEAD, n0 + _AHEAD, n0 + size + _AHEAD)

    def wait(dst, n):
        pltpu.make_async_copy(dst, dst, sems.at[n % _AHEAD]).wait()

    xa_cp = pltpu.make_async_copy(xa_hbm, xa_v, xsems.at[0])
    xb_cp = pltpu.make_async_copy(xb_hbm, xb_v, xsems.at[1])
    xa_cp.start()
    xb_cp.start()
    start_block(0, 0, 1)

    e_s[...] = (_iota((128, wide), 1) // _HG == _iota((128, wide), 0)).astype(_BF16)
    et_s[...] = (_iota((wide, 128), 0) // _HG == _iota((wide, 128), 1)).astype(_BF16)
    xa_cp.wait()
    xb_cp.wait()
    xa = xa_v[...].astype(_F32)
    for b in range(nb):
        xrow = jnp.broadcast_to(xa[b:b + 1], (_HG, dm)).astype(_BF16)
        for i in range(dm // 128):
            xr_s[i, b * _HG:(b + 1) * _HG, :] = xrow[:, i * 128:(i + 1) * 128]

    for n in range(1, _AHEAD):
        start_block(n, n, n + 1)

    def own_head(t):
        keep = _iota((rows, wide), 0) % _HG == _iota((rows, wide), 1) % _HG
        return jnp.where(keep, t, 0.0).astype(_BF16)

    def group_rows(w_v, j, g):
        return w_v[_ds(j * 128, 128), g * _HG:(g + 1) * _HG, :].reshape(wide, dh)

    zeros_q = tuple(jnp.zeros((rows, dh), _F32) for _ in range(ng))

    def qa_step(j, q):
        wait(wqa_v.at[_ds(j * 128, 128)], n_wqa + j)
        lhs = own_head(_dot(xr_s[j], e_s[...]))
        q = tuple(q[g] + _dot(lhs, group_rows(wqa_v, j, g)) for g in range(ng))
        refill(n_wqa, 4, j)
        return q

    qa = lax.fori_loop(0, 4, qa_step, zeros_q)
    qa = tuple(q.astype(_BF16) for q in qa)

    def qabs_step(j, carry):
        wait(wuk_v.at[_ds(j * 128, 128)], n_wuk + j)
        for g in range(ng):
            t = own_head(_dot_nt(qa[g], group_rows(wuk_v, j, g)))
            t = _dot(t, et_s[...]).astype(_BF16)
            for b in range(nb):
                qabs_s[j, b, g * _HG:(g + 1) * _HG, :] = t[b * _HG:(b + 1) * _HG]
        refill(n_wuk, 4, j)
        return carry

    lax.fori_loop(0, 4, qabs_step, None)

    def latent_batch(b, carry):
        q = jnp.concatenate([qabs_s[i, b] for i in range(4)], axis=-1)

        def step(jj, state):
            m, l, acc = state
            j = b * 4 + jj
            wait(ckv_v.at[j], n_ckv + j)
            c = ckv_v[j]
            s = _dot_nt(q, c) * scale
            m_new = jnp.maximum(m, jnp.max(s, axis=-1, keepdims=True))
            alpha = jnp.exp(m - m_new)
            p = jnp.exp(s - m_new)
            l = alpha * l + jnp.sum(p, axis=-1, keepdims=True)
            acc = alpha * acc + _dot(p.astype(_BF16), c)
            refill(n_ckv, 4 * nb, j)
            return m_new, l, acc

        init = (jnp.full((nh, 1), -jnp.inf, _F32), jnp.zeros((nh, 1), _F32),
                jnp.zeros((nh, ckv_v.shape[-1]), _F32))
        _, l, acc = lax.fori_loop(0, 4, step, init)
        ctxc = (acc / l).astype(_BF16)
        for i in range(4):
            for g in range(ng):
                ctxc_s[i, g, _ds(b * _HG, _HG), :] = (
                    ctxc[g * _HG:(g + 1) * _HG, i * 128:(i + 1) * 128])
        return carry

    lax.fori_loop(0, nb, latent_batch, None)

    def ctx_step(j, ctx):
        wait(wuv_v.at[_ds(j * 128, 128)], n_wuv + j)
        ctx = tuple(
            ctx[g] + _dot(own_head(_dot(ctxc_s[j, g], e_s[...])), group_rows(wuv_v, j, g))
            for g in range(ng))
        refill(n_wuv, 4, j)
        return ctx

    ctx = lax.fori_loop(0, 4, ctx_step, zeros_q)
    for g in range(ng):
        ctx_s[g] = ctx[g]

    def project_out(w_v, n0):
        def step(j, acc):
            shape = (rows, 8 * dh)
            keep = _iota(shape, 0) % _HG == (_iota(shape, 1) // dh) % 4 * 4 + j
            lhs = jnp.concatenate([ctx_s[g] for g in range(ng) for _ in range(4)], axis=-1)
            lhs = jnp.where(keep, lhs, 0.0).astype(_BF16)
            wait(w_v.at[j], n0 + j)
            acc = acc + _dot(lhs, w_v[j].reshape(8 * dh, dm))
            refill(n0, 4, j)
            return acc

        acc = lax.fori_loop(0, 4, step, jnp.zeros((rows, dm), _F32))
        return jnp.sum(acc.reshape(nb, _HG, dm), axis=1).astype(out_ref.dtype)

    out_ref[:, 0:dm] = project_out(woa_v, n_woa)

    xb = xb_v[...].astype(_F32)
    xb = jnp.concatenate(
        [jnp.broadcast_to(xb[b:b + 1], (8, dm)) for b in range(nb)], axis=0).astype(_BF16)

    def qb_step(j, carry):
        wait(wqb_v.at[j], n_wqb + j)
        q = _own_chunk(_dot(xb, wqb_v[j]))
        for b in range(nb):
            qb_s[b, j] = q[b * 8:(b + 1) * 8]
        refill(n_wqb, 4, j)
        return carry

    lax.fori_loop(0, 4, qb_step, None)

    def cache_batch(b, carry):
        j0 = b * 2 * nkb
        q = [qb_s[b, g].astype(_BF16) for g in range(nh // 8)]

        def slab(j, g):
            return kv_v[j % _SLOTS, g * 8:(g + 1) * 8].reshape(8 * _KEYS, dh)

        def k_step(jj, m):
            j = j0 + jj
            wait(kv_v.at[j % _SLOTS], n_cache + j)
            s = jnp.concatenate(
                [_own_chunk(_dot_nt(q[g], slab(j, g))) for g in range(nh // 8)], axis=0)
            s = s * scale
            sc_s[jj] = s
            refill(n_cache, 2 * nkb * nb - nkb, j)
            return jnp.maximum(m, s)

        m = lax.fori_loop(0, nkb, k_step, jnp.full((nh, _KEYS), -jnp.inf, _F32))
        m = jnp.broadcast_to(jnp.max(m, axis=-1, keepdims=True), (nh, _KEYS))

        def v_step(jj, state):
            l, acc = state
            j = j0 + nkb + jj
            p = jnp.exp(sc_s[jj] - m)
            shape = (8, 8 * _KEYS)
            keep = _iota(shape, 0) == _iota(shape, 1) // _KEYS
            lhs = [
                jnp.where(keep, jnp.concatenate([p[g * 8:(g + 1) * 8]] * 8, axis=-1), 0.0)
                .astype(_BF16) for g in range(nh // 8)]
            wait(kv_v.at[j % _SLOTS], n_cache + j)
            o = jnp.concatenate(
                [_dot(lhs[g], slab(j, g)) for g in range(nh // 8)], axis=0)
            refill(n_cache + nkb, 2 * nkb * nb - nkb, j - nkb)
            return l + p, acc + o

        zero = jnp.zeros((nh, dh), _F32)
        l, acc = lax.fori_loop(0, nkb, v_step, (zero, zero))
        o = acc / jnp.sum(l, axis=-1, keepdims=True)
        for g in range(ng):
            ctx_s[g, _ds(b * _HG, _HG), :] = o[g * _HG:(g + 1) * _HG]
        return carry

    lax.fori_loop(0, nb, cache_batch, None)
    out_ref[:, dm:2 * dm] = project_out(wob_v, n_wob)


@jax.jit
def pallas_concat_heads__compressed_kv_cla__mha_block_cached__decode_kernel(
    A_x: jax.Array,
    A_c_kv: jax.Array,
    A_w_q: jax.Array,
    A_w_uk: jax.Array,
    A_w_uv: jax.Array,
    A_w_o: jax.Array,
    B_x: jax.Array,
    B_k_cache: jax.Array,
    B_v_cache: jax.Array,
    B_wq: jax.Array,
    B_wo: jax.Array,
):
    nb, sq, dm = A_x.shape
    _, nh, sk, dh = B_k_cache.shape
    assert (nb, sq, dm, nh, sk, dh) == (4, 1, 512, 32, 4096, 128)
    assert A_c_kv.shape == (nb, sk, 512) and A_w_q.shape == (dm, nh, dh)
    rows, wide = nb * _HG, 128 * _HG
    vmem = pltpu.VMEM
    out = pl.pallas_call(
        _kernel,
        out_shape=jax.ShapeDtypeStruct((nb, 2 * dm), A_x.dtype),
        in_specs=[pl.BlockSpec(memory_space=pltpu.HBM)] * 11,
        out_specs=pl.BlockSpec(memory_space=pltpu.VMEM),
        scratch_shapes=[
            vmem((nb, dm), _BF16),
            vmem((nb, dm), _BF16),
            vmem(A_w_q.shape, _BF16),
            vmem(A_w_uk.shape, _BF16),
            vmem((4 * nb, sk // 4, A_c_kv.shape[-1]), _BF16),
            vmem(A_w_uv.shape, _BF16),
            vmem((4, 8, dh, dm), _BF16),
            vmem((4, dm, 8 * dh), _BF16),
            vmem((4, 8, dh, dm), _BF16),
            vmem((_SLOTS, nh, _KEYS, dh), _BF16),
            vmem((128, wide), _BF16),
            vmem((wide, 128), _BF16),
            vmem((dm // 128, rows, 128), _BF16),
            vmem((4, nb, nh, 128), _BF16),
            vmem((4, nh // _HG, rows, 128), _BF16),
            vmem((nh // _HG, rows, dh), _F32),
            vmem((nb, nh // 8, 8, dh), _F32),
            vmem((sk // _KEYS, nh, _KEYS), _F32),
            pltpu.SemaphoreType.DMA((_AHEAD,)),
            pltpu.SemaphoreType.DMA((2,)),
        ],
        compiler_params=pltpu.CompilerParams(
            vmem_limit_bytes=100 * 2**20,
            disable_bounds_checks=True,
        ),
    )(A_x.reshape(nb, dm), A_c_kv, A_w_q, A_w_uk, A_w_uv, A_w_o,
      B_x.reshape(nb, dm), B_k_cache, B_v_cache, B_wq, B_wo.reshape(nh, dh, dm))
    return out.reshape(nb, sq, 2 * dm)
```

```python
import functools

import jax
import jax.numpy as jnp
from jax import lax
import jax.experimental.pallas as pl
import jax.experimental.pallas.tpu as pltpu

_NT = (((1,), (1,)), ((), ()))
_PIECES = 64
_UNROLL = 32
_PRIORITY = (0, 1, 1, 1)
_AHEAD = 3
_SLOTS = 8
_HG = 16
_KEYS = 128
_F32 = jnp.float32
_BF16 = jnp.bfloat16


def _dot(a, b):
    return jnp.dot(a, b, preferred_element_type=_F32)


def _dot_nt(a, b):
    return lax.dot_general(a, b, _NT, preferred_element_type=_F32)


def _iota(shape, dim):
    return lax.broadcasted_iota(jnp.int32, shape, dim)


def _ds(start, size):
    return pl.ds(pl.multiple_of(start, size), size)


def _own_chunk(t):
    head = _iota((t.shape[0], 128), 0) % 8
    out = t[:, 0:128]
    for h in range(1, 8):
        out = jnp.where(head == h, t[:, h * 128:(h + 1) * 128], out)
    return out


def _kernel(
    xa_hbm, ckv_hbm, wqa_hbm, wuk_hbm, wuv_hbm, woa_hbm,
    xb_hbm, k_hbm, v_hbm, wqb_hbm, wob_hbm,
    out_ref,
    xa_v, xb_v, wqa_v, wuk_v, ckv_v, wuv_v, woa_v, wqb_v, wob_v, kv_v,
    e_s, et_s, xr_s, qabs_s, ctxc_s, ctx_s, qb_s, sc_s, sems, xsems,
):
    nb, nh, sk, dh = k_hbm.shape
    dm = xa_hbm.shape[-1]
    ng = nh // _HG
    rows = nb * _HG
    wide = 128 * _HG
    nkb = sk // _KEYS
    scale = dh ** -0.5

    def up_piece(hbm, vmem):
        def piece(j, t, r):
            u = t * (_UNROLL // 2) + r // 2
            sl = _ds(j * 128 + (r % 2) * 64 + u * 2, 2)
            return hbm.at[sl], vmem.at[sl]

        return piece

    def ckv_piece(j, t, r):
        u = t * (_UNROLL // 8) + r // 8
        src = _ds((r % 8) * 512 + (j % 4) * 128 + u * 16, 16)
        return ckv_hbm.at[j // 4, src], ckv_v.at[j, _ds((r % 8) * 128 + u * 16, 16)]

    def out_piece(hbm, vmem):
        def piece(j, t, r):
            sl = _ds((t * (_UNROLL // 8) + r // 8) * 16, 16)
            return hbm.at[(r % 8) * 4 + j, sl], vmem.at[j, r % 8, sl]

        return piece

    def wqb_piece(j, t, r):
        u = t * (_UNROLL // 8) + r // 8
        sl = _ds((r % 8) * 64 + (u // 2) * 16, 16)
        return (wqb_hbm.at[sl, _ds(j * 1024 + (u % 2) * 512, 512)],
                wqb_v.at[j, sl, _ds((u % 2) * 512, 512)])

    def cache_piece(hbm):
        def piece(j, t, r):
            n = _KEYS * nh // _PIECES
            u = t * (_UNROLL // nh) + r // nh
            src = _ds((j % nkb) * _KEYS + u * n, n)
            return (hbm.at[j // (2 * nkb), r % nh, src],
                    kv_v.at[j % _SLOTS, r % nh, _ds(u * n, n)])

        return piece

    def start(piece, j, n):
        def body(t, carry):
            for r in range(_UNROLL):
                src, dst = piece(j, t, r)
                pltpu.make_async_copy(src, dst, sems.at[n % _AHEAD]).start(
                    priority=_PRIORITY[r % len(_PRIORITY)])
            return carry

        lax.fori_loop(0, _PIECES // _UNROLL, body, None)

    def start_cache(j, n):
        is_k = (j // nkb) % 2 == 0
        pl.when(is_k)(lambda: start(cache_piece(k_hbm), j, n))
        pl.when(jnp.logical_not(is_k))(lambda: start(cache_piece(v_hbm), j, n))

    phases = (
        (4, functools.partial(start, up_piece(wqa_hbm, wqa_v))),
        (4, functools.partial(start, up_piece(wuk_hbm, wuk_v))),
        (4 * nb, functools.partial(start, ckv_piece)),
        (4, functools.partial(start, up_piece(wuv_hbm, wuv_v))),
        (4, functools.partial(start, out_piece(woa_hbm, woa_v))),
        (4, functools.partial(start, wqb_piece)),
        (2 * nkb * nb, start_cache),
        (4, functools.partial(start, out_piece(wob_hbm, wob_v))),
    )
    first = [sum(size for size, _ in phases[:k]) for k in range(len(phases))]
    n_wqa, n_wuk, n_ckv, n_wuv, n_woa, n_wqb, n_cache, n_wob = first

    def start_block(n, lo, hi):
        for (size, start_phase), n0 in zip(phases, first):
            if lo >= n0 and hi <= n0 + size:
                start_phase(n - n0, n)
            elif lo < n0 + size and hi > n0:
                pl.when((n >= n0) & (n < n0 + size))(
                    functools.partial(start_phase, n - n0, n))

    def refill(n0, size, j):
        start_block(n0 + j + _AHEAD, n0 + _AHEAD, n0 + size + _AHEAD)

    def wait(dst, n):
        pltpu.make_async_copy(dst, dst, sems.at[n % _AHEAD]).wait()

    xa_cp = pltpu.make_async_copy(xa_hbm, xa_v, xsems.at[0])
    xb_cp = pltpu.make_async_copy(xb_hbm, xb_v, xsems.at[1])
    xa_cp.start()
    xb_cp.start()
    start_block(0, 0, 1)

    e_s[...] = (_iota((128, wide), 1) // _HG == _iota((128, wide), 0)).astype(_BF16)
    et_s[...] = (_iota((wide, 128), 0) // _HG == _iota((wide, 128), 1)).astype(_BF16)
    xa_cp.wait()
    xb_cp.wait()
    xa = xa_v[...].astype(_F32)
    for b in range(nb):
        xrow = jnp.broadcast_to(xa[b:b + 1], (_HG, dm)).astype(_BF16)
        for i in range(dm // 128):
            xr_s[i, b * _HG:(b + 1) * _HG, :] = xrow[:, i * 128:(i + 1) * 128]

    for n in range(1, _AHEAD):
        start_block(n, n, n + 1)

    def own_head(t):
        keep = _iota((rows, wide), 0) % _HG == _iota((rows, wide), 1) % _HG
        return jnp.where(keep, t, 0.0).astype(_BF16)

    def group_rows(w_v, j, g):
        return w_v[_ds(j * 128, 128), g * _HG:(g + 1) * _HG, :].reshape(wide, dh)

    zeros_q = tuple(jnp.zeros((rows, dh), _F32) for _ in range(ng))

    def qa_step(j, q):
        wait(wqa_v.at[_ds(j * 128, 128)], n_wqa + j)
        lhs = own_head(_dot(xr_s[j], e_s[...]))
        q = tuple(q[g] + _dot(lhs, group_rows(wqa_v, j, g)) for g in range(ng))
        refill(n_wqa, 4, j)
        return q

    qa = lax.fori_loop(0, 4, qa_step, zeros_q)
    qa = tuple(q.astype(_BF16) for q in qa)

    def qabs_step(j, carry):
        wait(wuk_v.at[_ds(j * 128, 128)], n_wuk + j)
        for g in range(ng):
            t = own_head(_dot_nt(qa[g], group_rows(wuk_v, j, g)))
            t = _dot(t, et_s[...]).astype(_BF16)
            for b in range(nb):
                qabs_s[j, b, g * _HG:(g + 1) * _HG, :] = t[b * _HG:(b + 1) * _HG]
        refill(n_wuk, 4, j)
        return carry

    lax.fori_loop(0, 4, qabs_step, None)

    def latent_batch(b, carry):
        q = jnp.concatenate([qabs_s[i, b] for i in range(4)], axis=-1)

        def step(jj, state):
            m, l, acc = state
            j = b * 4 + jj
            wait(ckv_v.at[j], n_ckv + j)
            c = ckv_v[j]
            s = _dot_nt(q, c) * scale
            m_new = jnp.maximum(m, jnp.max(s, axis=-1, keepdims=True))
            alpha = jnp.exp(m - m_new)
            p = jnp.exp(s - m_new)
            l = alpha * l + jnp.sum(p, axis=-1, keepdims=True)
            acc = alpha * acc + _dot(p.astype(_BF16), c)
            refill(n_ckv, 4 * nb, j)
            return m_new, l, acc

        init = (jnp.full((nh, 1), -jnp.inf, _F32), jnp.zeros((nh, 1), _F32),
                jnp.zeros((nh, ckv_v.shape[-1]), _F32))
        _, l, acc = lax.fori_loop(0, 4, step, init)
        ctxc = (acc / l).astype(_BF16)
        for i in range(4):
            for g in range(ng):
                ctxc_s[i, g, _ds(b * _HG, _HG), :] = (
                    ctxc[g * _HG:(g + 1) * _HG, i * 128:(i + 1) * 128])
        return carry

    lax.fori_loop(0, nb, latent_batch, None)

    def ctx_step(j, ctx):
        wait(wuv_v.at[_ds(j * 128, 128)], n_wuv + j)
        ctx = tuple(
            ctx[g] + _dot(own_head(_dot(ctxc_s[j, g], e_s[...])), group_rows(wuv_v, j, g))
            for g in range(ng))
        refill(n_wuv, 4, j)
        return ctx

    ctx = lax.fori_loop(0, 4, ctx_step, zeros_q)
    ctx_s[...] = jnp.zeros(ctx_s.shape, _F32)
    for h in range(nh):
        for b in range(nb):
            row = b * _HG + h % _HG
            ctx_s[h, b:b + 1, :] = ctx[h // _HG][row:row + 1]

    def project_out(w_v, n0):
        def step(j, acc):
            lhs = jnp.concatenate([ctx_s[4 * t + j] for t in range(8)], axis=-1).astype(_BF16)
            wait(w_v.at[j], n0 + j)
            acc = acc + _dot(lhs, w_v[j].reshape(8 * dh, dm))
            refill(n0, 4, j)
            return acc

        acc = lax.fori_loop(0, 4, step, jnp.zeros((8, dm), _F32))
        return acc[0:nb].astype(out_ref.dtype)

    out_ref[:, 0:dm] = project_out(woa_v, n_woa)

    xb = xb_v[...].astype(_F32)
    xb = jnp.concatenate(
        [jnp.broadcast_to(xb[b:b + 1], (8, dm)) for b in range(nb)], axis=0).astype(_BF16)

    def qb_step(j, carry):
        wait(wqb_v.at[j], n_wqb + j)
        q = _own_chunk(_dot(xb, wqb_v[j]))
        for b in range(nb):
            qb_s[b, j] = q[b * 8:(b + 1) * 8]
        refill(n_wqb, 4, j)
        return carry

    lax.fori_loop(0, 4, qb_step, None)

    def cache_batch(b, carry):
        j0 = b * 2 * nkb
        q = [qb_s[b, g].astype(_BF16) for g in range(nh // 8)]

        def slab(j, g):
            return kv_v[j % _SLOTS, g * 8:(g + 1) * 8].reshape(8 * _KEYS, dh)

        def k_step(jj, m):
            j = j0 + jj
            wait(kv_v.at[j % _SLOTS], n_cache + j)
            s = jnp.concatenate(
                [_own_chunk(_dot_nt(q[g], slab(j, g))) for g in range(nh // 8)], axis=0)
            s = s * scale
            sc_s[jj] = s
            refill(n_cache, 2 * nkb * nb - nkb, j)
            return jnp.maximum(m, s)

        m = lax.fori_loop(0, nkb, k_step, jnp.full((nh, _KEYS), -jnp.inf, _F32))
        m = jnp.broadcast_to(jnp.max(m, axis=-1, keepdims=True), (nh, _KEYS))

        def v_step(jj, state):
            l, acc = state
            j = j0 + nkb + jj
            p = jnp.exp(sc_s[jj] - m)
            shape = (8, 8 * _KEYS)
            keep = _iota(shape, 0) == _iota(shape, 1) // _KEYS
            lhs = [
                jnp.where(keep, jnp.concatenate([p[g * 8:(g + 1) * 8]] * 8, axis=-1), 0.0)
                .astype(_BF16) for g in range(nh // 8)]
            wait(kv_v.at[j % _SLOTS], n_cache + j)
            o = jnp.concatenate(
                [_dot(lhs[g], slab(j, g)) for g in range(nh // 8)], axis=0)
            refill(n_cache + nkb, 2 * nkb * nb - nkb, j - nkb)
            return l + p, acc + o

        zero = jnp.zeros((nh, dh), _F32)
        l, acc = lax.fori_loop(0, nkb, v_step, (zero, zero))
        o = acc / jnp.sum(l, axis=-1, keepdims=True)
        for h in range(nh):
            ctx_s[h, pl.ds(b, 1), :] = o[h:h + 1]
        return carry

    lax.fori_loop(0, nb, cache_batch, None)
    out_ref[:, dm:2 * dm] = project_out(wob_v, n_wob)


@jax.jit
def pallas_concat_heads__compressed_kv_cla__mha_block_cached__decode_kernel(
    A_x: jax.Array,
    A_c_kv: jax.Array,
    A_w_q: jax.Array,
    A_w_uk: jax.Array,
    A_w_uv: jax.Array,
    A_w_o: jax.Array,
    B_x: jax.Array,
    B_k_cache: jax.Array,
    B_v_cache: jax.Array,
    B_wq: jax.Array,
    B_wo: jax.Array,
):
    nb, sq, dm = A_x.shape
    _, nh, sk, dh = B_k_cache.shape
    assert (nb, sq, dm, nh, sk, dh) == (4, 1, 512, 32, 4096, 128)
    assert A_c_kv.shape == (nb, sk, 512) and A_w_q.shape == (dm, nh, dh)
    rows, wide = nb * _HG, 128 * _HG
    vmem = pltpu.VMEM
    out = pl.pallas_call(
        _kernel,
        out_shape=jax.ShapeDtypeStruct((nb, 2 * dm), A_x.dtype),
        in_specs=[pl.BlockSpec(memory_space=pltpu.HBM)] * 11,
        out_specs=pl.BlockSpec(memory_space=pltpu.VMEM),
        scratch_shapes=[
            vmem((nb, dm), _BF16),
            vmem((nb, dm), _BF16),
            vmem(A_w_q.shape, _BF16),
            vmem(A_w_uk.shape, _BF16),
            vmem((4 * nb, sk // 4, A_c_kv.shape[-1]), _BF16),
            vmem(A_w_uv.shape, _BF16),
            vmem((4, 8, dh, dm), _BF16),
            vmem((4, dm, 8 * dh), _BF16),
            vmem((4, 8, dh, dm), _BF16),
            vmem((_SLOTS, nh, _KEYS, dh), _BF16),
            vmem((128, wide), _BF16),
            vmem((wide, 128), _BF16),
            vmem((dm // 128, rows, 128), _BF16),
            vmem((4, nb, nh, 128), _BF16),
            vmem((4, nh // _HG, rows, 128), _BF16),
            vmem((nh, 8, dh), _F32),
            vmem((nb, nh // 8, 8, dh), _F32),
            vmem((sk // _KEYS, nh, _KEYS), _F32),
            pltpu.SemaphoreType.DMA((_AHEAD,)),
            pltpu.SemaphoreType.DMA((2,)),
        ],
        compiler_params=pltpu.CompilerParams(
            vmem_limit_bytes=100 * 2**20,
            disable_bounds_checks=True,
        ),
    )(A_x.reshape(nb, dm), A_c_kv, A_w_q, A_w_uk, A_w_uv, A_w_o,
      B_x.reshape(nb, dm), B_k_cache, B_v_cache, B_wq, B_wo.reshape(nh, dh, dm))
    return out.reshape(nb, sq, 2 * dm)
```

```python
import functools

import jax
import jax.numpy as jnp
from jax import lax
import jax.experimental.pallas as pl
import jax.experimental.pallas.tpu as pltpu

_NT = (((1,), (1,)), ((), ()))
_RUN = 32
_PRIORITY = (1, 1, 1, 0)
_AHEAD = 3
_SLOTS = 8
_HG = 16
_KEYS = 128
_TAIL = 6
_F32 = jnp.float32
_BF16 = jnp.bfloat16


def _dot(a, b):
    return jnp.dot(a, b, preferred_element_type=_F32)


def _dot_nt(a, b):
    return lax.dot_general(a, b, _NT, preferred_element_type=_F32)


def _iota(shape, dim):
    return lax.broadcasted_iota(jnp.int32, shape, dim)


def _ds(start, size):
    return pl.ds(pl.multiple_of(start, size), size)


def _own_chunk(t):
    head = _iota((t.shape[0], 128), 0) % 8
    out = t[:, 0:128]
    for h in range(1, 8):
        out = jnp.where(head == h, t[:, h * 128:(h + 1) * 128], out)
    return out


def _own_head(t):
    keep = _iota(t.shape, 0) % _HG == _iota(t.shape, 1) % _HG
    return jnp.where(keep, t, 0.0).astype(_BF16)


def _kernel(
    xa_hbm, ckv_hbm, wqa_hbm, wuk_hbm, wuv_hbm, woa_hbm,
    xb_hbm, k_hbm, v_hbm, wqb_hbm, wob_hbm,
    out_ref,
    xa_v, xb_v, wqa_v, wuk_v, ckv_v, wuv_v, woa_v, wqb_v, wob_v, kv_v,
    e_s, et_s, xr_s, qabs_s, ctxc_s, ctx_s, qb_s, sc_s, sems, xsems,
):
    nb, nh, sk, dh = k_hbm.shape
    dm = xa_hbm.shape[-1]
    ng = nh // _HG
    rows = nb * _HG
    wide = 128 * _HG
    nkb = sk // _KEYS
    scale = dh ** -0.5

    def up_piece(hbm, vmem):
        def piece(j, t, r):
            sl = _ds(j * 128 + (r % 2) * 64 + t * _RUN + (r // 2) * 2, 2)
            return hbm.at[sl], vmem.at[sl]

        return piece

    def ckv_piece(j, t, r):
        off = (t * (_RUN // 8) + r // 8) * 16
        src = _ds((r % 8) * 512 + (j % 4) * 128 + off, 16)
        return ckv_hbm.at[j // 4, src], ckv_v.at[j, _ds((r % 8) * 128 + off, 16)]

    def out_piece(hbm, vmem):
        def piece(j, t, r):
            sl = _ds((t * (_RUN // 8) + r // 8) * 16, 16)
            return hbm.at[(r % 8) * 4 + j, sl], vmem.at[j, r % 8, sl]

        return piece

    def wqb_piece(j, t, r):
        sl = _ds((r % 8) * 64 + (t * (_RUN // 16) + r // 16) * 16, 16)
        col = (r // 8) % 2 * 512
        return (wqb_hbm.at[sl, _ds(j * 1024 + col, 512)],
                wqb_v.at[j, sl, pl.ds(col, 512)])

    def cache_piece(hbm):
        def piece(j, t, r):
            n = _KEYS // 2
            return (hbm.at[j // (2 * nkb), r, _ds((j % nkb) * _KEYS + t * n, n)],
                    kv_v.at[j % _SLOTS, r, _ds(t * n, n)])

        return piece

    def start_dma(src, dst, n, r):
        pltpu.make_async_copy(src, dst, sems.at[n % _AHEAD]).start(
            priority=_PRIORITY[r % len(_PRIORITY)])

    def start(piece, j, n):
        def run(t, carry):
            for r in range(_RUN):
                start_dma(*piece(j, t, r), n, r)
            return carry

        lax.fori_loop(0, 2, run, None)

    def start_cache(j, n):
        is_k = (j // nkb) % 2 == 0
        pl.when(is_k)(lambda: start(cache_piece(k_hbm), j, n))
        pl.when(jnp.logical_not(is_k))(lambda: start(cache_piece(v_hbm), j, n))

    def start_tail(h0, h1, j, n):
        del j
        for r in range((h1 - h0) * 8):
            h, sl = h0 + r % (h1 - h0), pl.ds(r // (h1 - h0) * 16, 16)
            start_dma(wob_hbm.at[h * 4 + 3, sl], wob_v.at[3, h, sl], n, r)

    phases = (
        (4, functools.partial(start, up_piece(wqa_hbm, wqa_v))),
        (4, functools.partial(start, up_piece(wuk_hbm, wuk_v))),
        (4 * nb, functools.partial(start, ckv_piece)),
        (4, functools.partial(start, up_piece(wuv_hbm, wuv_v))),
        (4, functools.partial(start, out_piece(woa_hbm, woa_v))),
        (4, functools.partial(start, wqb_piece)),
        (2 * nkb * nb, start_cache),
        (3, functools.partial(start, out_piece(wob_hbm, wob_v))),
        (1, functools.partial(start_tail, 0, _TAIL)),
        (1, functools.partial(start_tail, _TAIL, 8)),
    )
    first = [sum(size for size, _ in phases[:k]) for k in range(len(phases))]
    n_wqa, n_wuk, n_ckv, n_wuv, n_woa, n_wqb, n_cache, n_wob = first[:8]

    def start_block(n, lo, hi):
        for (size, start_phase), n0 in zip(phases, first):
            if lo >= n0 and hi <= n0 + size:
                start_phase(n - n0, n)
            elif lo < n0 + size and hi > n0:
                pl.when((n >= n0) & (n < n0 + size))(
                    functools.partial(start_phase, n - n0, n))

    def refill(n0, size, j):
        start_block(n0 + j + _AHEAD, n0 + _AHEAD, n0 + size + _AHEAD)

    def wait(dst, n):
        pltpu.make_async_copy(dst, dst, sems.at[n % _AHEAD]).wait()

    xa_cp = pltpu.make_async_copy(xa_hbm, xa_v, xsems.at[0])
    xb_cp = pltpu.make_async_copy(xb_hbm, xb_v, xsems.at[1])
    xa_cp.start()
    xb_cp.start()
    start_block(0, 0, 1)

    e_s[...] = (_iota((128, wide), 1) // _HG == _iota((128, wide), 0)).astype(_BF16)
    et_s[...] = (_iota((wide, 128), 0) // _HG == _iota((wide, 128), 1)).astype(_BF16)
    xa_cp.wait()
    xb_cp.wait()
    xa = xa_v[...].astype(_F32)
    for b in range(nb):
        xrow = jnp.broadcast_to(xa[b:b + 1], (_HG, dm)).astype(_BF16)
        for i in range(dm // 128):
            xr_s[i, b * _HG:(b + 1) * _HG, :] = xrow[:, i * 128:(i + 1) * 128]

    for n in range(1, _AHEAD):
        start_block(n, n, n + 1)

    def group_rows(w_v, j, g):
        return w_v[_ds(j * 128, 128), g * _HG:(g + 1) * _HG, :].reshape(wide, dh)

    zeros_q = tuple(jnp.zeros((rows, dh), _F32) for _ in range(ng))

    def qa_step(j, q):
        wait(wqa_v.at[_ds(j * 128, 128)], n_wqa + j)
        lhs = _own_head(_dot(xr_s[j], e_s[...]))
        q = tuple(q[g] + _dot(lhs, group_rows(wqa_v, j, g)) for g in range(ng))
        refill(n_wqa, 4, j)
        return q

    qa = lax.fori_loop(0, 4, qa_step, zeros_q)
    qa = tuple(q.astype(_BF16) for q in qa)

    def qabs_step(j, carry):
        wait(wuk_v.at[_ds(j * 128, 128)], n_wuk + j)
        for g in range(ng):
            t = _own_head(_dot_nt(qa[g], group_rows(wuk_v, j, g)))
            t = _dot(t, et_s[...]).astype(_BF16)
            for b in range(nb):
                qabs_s[j, b, g * _HG:(g + 1) * _HG, :] = t[b * _HG:(b + 1) * _HG]
        refill(n_wuk, 4, j)
        return carry

    lax.fori_loop(0, 4, qabs_step, None)

    def latent_batch(b, carry):
        q = jnp.concatenate([qabs_s[i, b] for i in range(4)], axis=-1)

        def step(jj, state):
            m, l, acc = state
            j = b * 4 + jj
            wait(ckv_v.at[j], n_ckv + j)
            c = ckv_v[j]
            s = _dot_nt(q, c) * scale
            m_new = jnp.maximum(m, jnp.max(s, axis=-1, keepdims=True))
            alpha = jnp.exp(m - m_new)
            p = jnp.exp(s - m_new)
            l = alpha * l + jnp.sum(p, axis=-1, keepdims=True)
            acc = alpha * acc + _dot(p.astype(_BF16), c)
            refill(n_ckv, 4 * nb, j)
            return m_new, l, acc

        init = (jnp.full((nh, 1), -jnp.inf, _F32), jnp.zeros((nh, 1), _F32),
                jnp.zeros((nh, ckv_v.shape[-1]), _F32))
        _, l, acc = lax.fori_loop(0, 4, step, init)
        ctxc = (acc / l).astype(_BF16)
        for i in range(4):
            for g in range(ng):
                ctxc_s[i, g, _ds(b * _HG, _HG), :] = (
                    ctxc[g * _HG:(g + 1) * _HG, i * 128:(i + 1) * 128])
        return carry

    lax.fori_loop(0, nb, latent_batch, None)

    def ctx_step(j, ctx):
        wait(wuv_v.at[_ds(j * 128, 128)], n_wuv + j)
        ctx = tuple(
            ctx[g] + _dot(_own_head(_dot(ctxc_s[j, g], e_s[...])), group_rows(wuv_v, j, g))
            for g in range(ng))
        refill(n_wuv, 4, j)
        return ctx

    ctx = lax.fori_loop(0, 4, ctx_step, zeros_q)
    ctx_s[...] = jnp.zeros(ctx_s.shape, _F32)
    for h in range(nh):
        for b in range(nb):
            row = b * _HG + h % _HG
            ctx_s[h, b:b + 1, :] = ctx[h // _HG][row:row + 1]

    def project_out(w_v, j, h0, h1, n):
        lhs = jnp.concatenate([ctx_s[4 * h + j] for h in range(h0, h1)], axis=-1)
        lhs = lhs.astype(_BF16)
        wait(w_v.at[j, h0:h1], n)
        return _dot(lhs, w_v[j, h0:h1].reshape((h1 - h0) * dh, dm))

    def outa_step(j, acc):
        acc = acc + project_out(woa_v, j, 0, 8, n_woa + j)
        refill(n_woa, 4, j)
        return acc

    outa = lax.fori_loop(0, 4, outa_step, jnp.zeros((8, dm), _F32))
    out_ref[:, 0:dm] = outa[0:nb].astype(out_ref.dtype)

    xb = xb_v[...].astype(_F32)
    xb = jnp.concatenate(
        [jnp.broadcast_to(xb[b:b + 1], (8, dm)) for b in range(nb)], axis=0).astype(_BF16)

    def qb_step(j, carry):
        wait(wqb_v.at[j], n_wqb + j)
        q = _own_chunk(_dot(xb, wqb_v[j]))
        for b in range(nb):
            qb_s[b, j] = q[b * 8:(b + 1) * 8]
        refill(n_wqb, 4, j)
        return carry

    lax.fori_loop(0, 4, qb_step, None)

    def cache_batch(b, carry):
        j0 = b * 2 * nkb
        q = [qb_s[b, g].astype(_BF16) for g in range(nh // 8)]

        def slab(j, g):
            return kv_v[j % _SLOTS, g * 8:(g + 1) * 8].reshape(8 * _KEYS, dh)

        def k_step(jj, m):
            j = j0 + jj
            wait(kv_v.at[j % _SLOTS], n_cache + j)
            s = jnp.concatenate(
                [_own_chunk(_dot_nt(q[g], slab(j, g))) for g in range(nh // 8)], axis=0)
            s = s * scale
            sc_s[jj] = s
            refill(n_cache, 2 * nkb * nb - nkb, j)
            return jnp.maximum(m, s)

        m = lax.fori_loop(0, nkb, k_step, jnp.full((nh, _KEYS), -jnp.inf, _F32))
        m = jnp.broadcast_to(jnp.max(m, axis=-1, keepdims=True), (nh, _KEYS))

        def v_step(jj, state):
            l, acc = state
            j = j0 + nkb + jj
            p = jnp.exp(sc_s[jj] - m)
            shape = (8, 8 * _KEYS)
            keep = _iota(shape, 0) == _iota(shape, 1) // _KEYS
            lhs = [
                jnp.where(keep, jnp.concatenate([p[g * 8:(g + 1) * 8]] * 8, axis=-1), 0.0)
                .astype(_BF16) for g in range(nh // 8)]
            wait(kv_v.at[j % _SLOTS], n_cache + j)
            o = jnp.concatenate(
                [_dot(lhs[g], slab(j, g)) for g in range(nh // 8)], axis=0)
            refill(n_cache + nkb, 2 * nkb * nb - nkb, j - nkb)
            return l + p, acc + o

        zero = jnp.zeros((nh, dh), _F32)
        l, acc = lax.fori_loop(0, nkb, v_step, (zero, zero))
        o = acc / jnp.sum(l, axis=-1, keepdims=True)
        for h in range(nh):
            ctx_s[h, pl.ds(b, 1), :] = o[h:h + 1]
        return carry

    lax.fori_loop(0, nb, cache_batch, None)

    outb = jnp.zeros((8, dm), _F32)
    blocks = ((0, 0, 8), (1, 0, 8), (2, 0, 8), (3, 0, _TAIL), (3, _TAIL, 8))
    for i, (j, h0, h1) in enumerate(blocks):
        outb = outb + project_out(wob_v, j, h0, h1, n_wob + i)
        refill(n_wob + i, 1, 0)
    out_ref[:, dm:2 * dm] = outb[0:nb].astype(out_ref.dtype)


@jax.jit
def pallas_concat_heads__compressed_kv_cla__mha_block_cached__decode_kernel(
    A_x: jax.Array,
    A_c_kv: jax.Array,
    A_w_q: jax.Array,
    A_w_uk: jax.Array,
    A_w_uv: jax.Array,
    A_w_o: jax.Array,
    B_x: jax.Array,
    B_k_cache: jax.Array,
    B_v_cache: jax.Array,
    B_wq: jax.Array,
    B_wo: jax.Array,
):
    nb, sq, dm = A_x.shape
    _, nh, sk, dh = B_k_cache.shape
    dc = A_c_kv.shape[-1]
    assert (nb, sq, dm, nh, sk, dh, dc) == (4, 1, 512, 32, 4096, 128, 512)
    assert A_c_kv.shape == (nb, sk, dc) and A_w_q.shape == (dm, nh, dh)
    rows, wide = nb * _HG, 128 * _HG
    vmem = pltpu.VMEM
    out = pl.pallas_call(
        _kernel,
        out_shape=jax.ShapeDtypeStruct((nb, 2 * dm), A_x.dtype),
        in_specs=[pl.BlockSpec(memory_space=pltpu.HBM)] * 11,
        out_specs=pl.BlockSpec(memory_space=pltpu.VMEM),
        scratch_shapes=[
            vmem((nb, dm), _BF16),
            vmem((nb, dm), _BF16),
            vmem(A_w_q.shape, _BF16),
            vmem(A_w_uk.shape, _BF16),
            vmem((4 * nb, sk // 4, dc), _BF16),
            vmem(A_w_uv.shape, _BF16),
            vmem((4, 8, dh, dm), _BF16),
            vmem((4, dm, 8 * dh), _BF16),
            vmem((4, 8, dh, dm), _BF16),
            vmem((_SLOTS, nh, _KEYS, dh), _BF16),
            vmem((128, wide), _BF16),
            vmem((wide, 128), _BF16),
            vmem((dm // 128, rows, 128), _BF16),
            vmem((dc // 128, nb, nh, 128), _BF16),
            vmem((dc // 128, nh // _HG, rows, 128), _BF16),
            vmem((nh, 8, dh), _F32),
            vmem((nb, nh // 8, 8, dh), _F32),
            vmem((sk // _KEYS, nh, _KEYS), _F32),
            pltpu.SemaphoreType.DMA((_AHEAD,)),
            pltpu.SemaphoreType.DMA((2,)),
        ],
        compiler_params=pltpu.CompilerParams(
            vmem_limit_bytes=100 * 2**20,
            disable_bounds_checks=True,
        ),
    )(A_x.reshape(nb, dm), A_c_kv, A_w_q, A_w_uk, A_w_uv, A_w_o,
      B_x.reshape(nb, dm), B_k_cache, B_v_cache, B_wq, B_wo.reshape(nh, dh, dm))
    return out.reshape(nb, sq, 2 * dm)
```
